```python
import os as _os
_os.environ.setdefault("JAX_PLATFORMS", "cpu")
import jax
import jax.numpy as jnp

def _softmax(x, axis=-1):
    return jax.nn.softmax(x, axis=axis)
def _gelu(x):
    return jax.nn.gelu(x, approximate=True)
def _silu(x):
    return jax.nn.silu(x)
def _sigmoid(x):
    return jax.nn.sigmoid(x)
def _layernorm(x, axis=-1, eps=1e-5):
    m = jnp.mean(x, axis=axis, keepdims=True)
    v = jnp.var(x, axis=axis, keepdims=True)
    return (x - m) / jnp.sqrt(v + eps)
def _scatter_add(tgt, idx, src, axis=0):
    return tgt.at[idx].add(src)
def _segment_sum(src, seg, n):
    return jax.ops.segment_sum(src, seg, n)
class _Rng:
    def __init__(self, key):
        self._k = key
    def _next(self):
        self._k, sub = jax.random.split(self._k)
        return sub
    def normal(self, shape):
        return jax.random.normal(self._next(), shape, dtype=jnp.bfloat16)
    def randint(self, lo, hi, shape):
        return jax.random.randint(self._next(), shape, lo, hi, dtype=jnp.int32)
    def uniform(self, shape, lo=0.0, hi=1.0):
        return jax.random.uniform(self._next(), shape, jnp.bfloat16, lo, hi)
    def permutation(self, n):
        return jax.random.permutation(self._next(), n)


kernel_name = 'parallel_sum__softmax_full_mha__moe_arch_mod__prompt'

def setup_inputs():
    _rng = _Rng(jax.random.key(int.from_bytes(__import__("os").urandom(4), "little")))
    _w = (lambda a: (lambda t: t.astype(jnp.bfloat16) if jnp.issubdtype(t.dtype, jnp.floating) else t)(jnp.asarray(a)))
    def _A_setup():
        B, S, D = 1, 2048, 512
        return {
            "x": _w((lambda *s: _rng.normal(s) * 0.05)(B, S, D)),
            "wqkv": _w((lambda *s: _rng.normal(s) * 0.1)(D, 3 * D)),
            "wo": _w((lambda *s: _rng.normal(s) * 0.05)(D, D)),
        }
    _A_in = _A_setup()

    def _B_setup():
        B, S, D, F, C = 1, 2048, 512, 1792, 1
        return {
            "x": _w((lambda *s: _rng.normal(s) * 0.05)(B, S, D)),
            "w_r": _w((lambda *s: _rng.normal(s) * 1.6)(D)),
            "w_gate": _w((lambda *s: _rng.normal(s) * 0.1)(D, F)),
            "w_up": _w((lambda *s: _rng.normal(s) * 0.1)(D, F)),
            "w_down": _w((lambda *s: _rng.normal(s) * 0.1)(F, D)),
        }
    _B_in = _B_setup()

    return {
        "A_x": _A_in["x"],
        "A_wqkv": _A_in["wqkv"],
        "A_wo": _A_in["wo"],
        "B_x": _B_in["x"],
        "B_w_r": _B_in["w_r"],
        "B_w_gate": _B_in["w_gate"],
        "B_w_up": _B_in["w_up"],
        "B_w_down": _B_in["w_down"],
    }

def reference(A_x, A_wqkv, A_wo, B_x, B_w_r, B_w_gate, B_w_up, B_w_down):
    def _A_ref(x, wqkv, wo):
        B, S, D = x.shape
        H = 32; Dh = D // H
        qkv = (lambda x, *d: x.transpose(*d))((x @ wqkv).reshape(B, S, 3, H, Dh), 2, 0, 3, 1, 4)
        q, k, v = qkv[0], qkv[1], qkv[2]
        scale = Dh ** -0.5
        scores = jnp.einsum("bhqd,bhkd->bhqk", q, k) * scale
        p = _softmax(scores, axis=-1)
        o = jnp.einsum("bhqk,bhkd->bhqd", p, v)
        return (lambda x, *d: x.transpose(*d))(o, 0, 2, 1, 3).reshape(B, S, D) @ wo

    def _B_ref(x, w_r, w_gate, w_up, w_down):
        B, S, D = x.shape
        C = 1
        r = x @ w_r
        idx = jnp.argsort(-r, axis=-1)[:, :C]
        idx_e = jnp.repeat(idx.reshape(B, C, 1), D, axis=2)
        x_sel = jnp.take_along_axis(x, idx_e, axis=1)
        g = _silu(x_sel @ w_gate)
        u = x_sel @ w_up
        y = (g * u) @ w_down
        r_sel = _sigmoid(jnp.take_along_axis(r, idx, axis=1))
        y = y * r_sel.reshape(B, C, 1)
        b_off = (jnp.arange(B) * S).reshape(B, 1)
        flat_idx = (idx + b_off).reshape(B * C)
        zero = (x * 0.0).reshape(B * S, D)
        upd = _scatter_add(zero, flat_idx, y.reshape(B * C, D), axis=0)
        return x + upd.reshape(B, S, D)

    x = A_x
    xn = _layernorm(x, axis=-1)
    return x + _A_ref(xn, A_wqkv, A_wo) + _B_ref(xn, B_w_r, B_w_gate, B_w_up, B_w_down)
```

```python
import functools
import numpy as np
import jax
import jax.numpy as jnp
import jax.experimental.pallas as pl
import jax.experimental.pallas.tpu as pltpu

_S, _D, _H, _DH, _F = 2048, 512, 32, 16, 1792
_BQ = 512
_CK = 128
_SKEW = 2
_RC = 512
_LOG2E = 1.4426950408889634
_L_MAX = float(2.0 ** 64)

f32 = jnp.float32
bf16 = jnp.bfloat16


def _rb(x):
    return x.astype(bf16).astype(f32)


def _kernel(x_ref, wqkv_ref, wo_ref, wr_ref, wg_hbm, wu_hbm, wd_hbm, o_ref,
            xn_s, k_s, qt_s, vt_s, ot_s, wt_s, wg_s, wu_s, wd_s, sems):
    S, D, H, DH, F, BQ, CK = _S, _D, _H, _DH, _F, _BQ, _CK
    nq, nc = S // BQ, S // CK
    cps = [pltpu.make_async_copy(wg_hbm, wg_s, sems.at[0]),
           pltpu.make_async_copy(wu_hbm, wu_s, sems.at[1]),
           pltpu.make_async_copy(wd_hbm, wd_s, sems.at[2])]
    for c in cps:
        c.start()

    wt_s[0:D, :] = wqkv_ref[:, 0:D].astype(f32).T.astype(bf16)
    wt_s[D:2 * D, :] = wqkv_ref[:, 2 * D:3 * D].astype(f32).T.astype(bf16)
    wt_s[2 * D:2 * D + 16, :] = jnp.broadcast_to(wr_ref[...].reshape(1, D), (16, D))
    eps_b = float(np.float32(np.asarray(1e-5, dtype=jnp.bfloat16)))
    qscale = (DH ** -0.5) * _LOG2E
    rparts = []
    for i in range(S // _RC):
        rows = pl.ds(i * _RC, _RC)
        xf = x_ref[rows, :].astype(f32)
        mean = jnp.sum(xf, axis=-1, keepdims=True) * (1.0 / D)
        xc0 = xf - mean
        var = jnp.sum(xc0 * xc0, axis=-1, keepdims=True) * (1.0 / D)
        xc = _rb(xf - _rb(mean))
        den = _rb(jnp.sqrt(_rb(_rb(var) + eps_b)))
        xn = (xc / den).astype(bf16)
        xn_s[rows, :] = xn
        qv = jax.lax.dot_general(wt_s[...], xn, (((1,), (1,)), ((), ())),
                                 preferred_element_type=f32)
        qt_s[:, rows] = (qv[0:D] * qscale).astype(bf16)
        vt_s[:, rows] = qv[D:2 * D].astype(bf16)
        rparts.append(qv[2 * D:2 * D + 8])
        k_s[rows, :] = jnp.dot(xn, wqkv_ref[:, D:2 * D], preferred_element_type=f32).astype(bf16)
    r = _rb(jnp.concatenate(rparts, axis=1))
    rmax = jnp.max(r)
    lane = jax.lax.broadcasted_iota(jnp.int32, (8, S), 1)
    idx = jnp.min(jnp.where(r == rmax, lane, S - 1))

    def qtile(h, j):
        q16 = qt_s[pl.ds(pl.multiple_of(h * DH, DH), DH), pl.ds(j * BQ, BQ)]
        row = jax.lax.broadcasted_iota(jnp.int32, (128, BQ), 0)
        qf = jnp.concatenate([q16] * 8, axis=0)
        return jnp.where((row // DH) == (h % 8), qf, jnp.zeros_like(qf))

    def head(h, bad):
        goff = pl.multiple_of((h // 8) * 128, 128)
        hoff = pl.multiple_of(h * DH, DH)
        work = [(j, c) for j in range(nq) for c in range(nc)]
        pend = []
        qm = m = l = acc = None
        for n in range(len(work) + _SKEW):
            if n < len(work):
                j, c = work[n]
                if c == 0:
                    qm = qtile(h, j)
                s = jnp.dot(k_s[pl.ds(c * CK, CK), pl.ds(goff, 128)], qm, preferred_element_type=f32)
                if c == 0:
                    m = jnp.max(jnp.max(s.reshape(CK // 8, 8, BQ), axis=0), axis=0, keepdims=True)
                p = jnp.exp2(s - m)
                lc = jnp.sum(p.reshape(CK // 8, 8, BQ), axis=0)
                l = lc if c == 0 else l + lc
                pend.append((p.astype(bf16), l))
            if n >= _SKEW:
                j, c = work[n - _SKEW]
                pp, lp = pend[n - _SKEW]
                o = jnp.dot(vt_s[pl.ds(hoff, DH), pl.ds(c * CK, CK)], pp, preferred_element_type=f32)
                acc = o if c == 0 else acc + o
                if c == nc - 1:
                    lt = jnp.sum(lp, axis=0, keepdims=True)
                    on = acc * (1.0 / lt)
                    ot_s[pl.ds(hoff, DH), pl.ds(j * BQ, BQ)] = on.astype(bf16)
                    ok = jnp.logical_and(lt < _L_MAX, jnp.max(jnp.abs(acc), axis=0, keepdims=True) < np.inf)
                    bad = jnp.maximum(bad, jnp.where(ok, 0.0, 1.0))
        return bad

    bad = jax.lax.fori_loop(0, H, head, jnp.zeros((1, BQ), f32))

    @pl.when(jnp.max(bad) > 0.0)
    def _():
        def blk(n, carry):
            h = n // nq
            j = n % nq
            goff = pl.multiple_of((h // 8) * 128, 128)
            hoff = pl.multiple_of(h * DH, DH)
            joff = pl.multiple_of(j * BQ, BQ)
            q16 = qt_s[pl.ds(hoff, DH), pl.ds(joff, BQ)]
            row = jax.lax.broadcasted_iota(jnp.int32, (128, BQ), 0)
            qf = jnp.concatenate([q16] * 8, axis=0)
            qm = jnp.where((row // DH) == (h % 8), qf, jnp.zeros_like(qf))

            def scores(c):
                coff = pl.multiple_of(c * CK, CK)
                return coff, jnp.dot(k_s[pl.ds(coff, CK), pl.ds(goff, 128)], qm, preferred_element_type=f32)

            def p1(c, m):
                _, s = scores(c)
                return jnp.maximum(m, jnp.max(s, axis=0, keepdims=True))
            m = jax.lax.fori_loop(0, nc, p1, jnp.full((1, BQ), -np.inf, f32))

            def p2(c, la):
                l, acc = la
                coff, s = scores(c)
                p = jnp.exp2(s - m)
                l = l + jnp.sum(p, axis=0, keepdims=True)
                acc = acc + jnp.dot(vt_s[pl.ds(hoff, DH), pl.ds(coff, CK)], p.astype(bf16),
                                    preferred_element_type=f32)
                return l, acc
            l, acc = jax.lax.fori_loop(0, nc, p2, (jnp.zeros((1, BQ), f32), jnp.zeros((DH, BQ), f32)))
            ot_s[pl.ds(hoff, DH), pl.ds(joff, BQ)] = (acc * (1.0 / l)).astype(bf16)
            return carry
        jax.lax.fori_loop(0, H * nq, blk, 0)

    for c in cps:
        c.wait()
    base = pl.multiple_of((idx // 16) * 16, 16)
    xt = xn_s[pl.ds(base, 16), :]
    row = jax.lax.broadcasted_iota(jnp.int32, (16, D), 0)
    xt = jnp.where(row == idx - base, xt, jnp.zeros_like(xt))
    g = _rb(jnp.dot(xt, wg_s[...], preferred_element_type=f32))
    u = _rb(jnp.dot(xt, wu_s[...], preferred_element_type=f32))
    hh = (_rb(g * jax.nn.sigmoid(g)) * u).astype(bf16)
    y = _rb(jnp.dot(hh, wd_s[...], preferred_element_type=f32)) * _rb(jax.nn.sigmoid(jnp.full((1, D), rmax, f32)))

    for i in range(S // _RC):
        rows = pl.ds(i * _RC, _RC)
        a = jax.lax.dot_general(ot_s[:, rows], wo_ref[...], (((0,), (0,)), ((), ())),
                                preferred_element_type=f32)
        o_ref[rows, :] = (x_ref[rows, :].astype(f32) + a + xn_s[rows, :].astype(f32)).astype(bf16)
    rows = pl.ds(base, 16)
    o_ref[rows, :] = (o_ref[rows, :].astype(f32) + y).astype(bf16)


@jax.jit
def pallas_parallel_sum__softmax_full_mha__moe_arch_mod__prompt_kernel(
    A_x, A_wqkv, A_wo, B_x, B_w_r, B_w_gate, B_w_up, B_w_down,
):
    S, D, F = _S, _D, _F
    vm = pl.BlockSpec(memory_space=pltpu.VMEM)
    hb = pl.BlockSpec(memory_space=pl.ANY)
    out = pl.pallas_call(
        _kernel,
        out_shape=jax.ShapeDtypeStruct((S, D), bf16),
        in_specs=[vm, vm, vm, vm, hb, hb, hb],
        out_specs=vm,
        scratch_shapes=[
            pltpu.VMEM((S, D), bf16),
            pltpu.VMEM((S, D), bf16),
            pltpu.VMEM((D, S), bf16),
            pltpu.VMEM((D, S), bf16),
            pltpu.VMEM((D, S), bf16),
            pltpu.VMEM((2 * D + 16, D), bf16),
            pltpu.VMEM((D, F), bf16),
            pltpu.VMEM((D, F), bf16),
            pltpu.VMEM((F, D), bf16),
            pltpu.SemaphoreType.DMA((3,)),
        ],
        compiler_params=pltpu.CompilerParams(vmem_limit_bytes=100 * 1024 * 1024),
    )(A_x.reshape(S, D), A_wqkv, A_wo, B_w_r, B_w_gate, B_w_up, B_w_down)
    return out.reshape(1, S, D)
```

```python
import functools

import numpy as np
import jax
import jax.numpy as jnp
import jax.experimental.pallas as pl
import jax.experimental.pallas.tpu as pltpu

_S, _D, _H, _DH, _F = 2048, 512, 32, 16, 1792
_BQ = 512
_CK = 128
_MK = 32
_SKEW = 2
_HPI = 2
_RC = 512
_KC = 128
_OC = 256
_LOG2E = 1.4426950408889634
_L_MAX = float(2.0 ** 120)
_EPS_BF16 = float(np.float32(np.asarray(1e-5, dtype=jnp.bfloat16)))

f32 = jnp.float32
bf16 = jnp.bfloat16


def _rb(x):
    return x.astype(bf16).astype(f32)


def _dot(a, b):
    return jnp.dot(a, b, preferred_element_type=f32)


def _kernel(x_hbm, wqkv_hbm, wo_hbm, wr_ref, wg_hbm, wu_hbm, wd_hbm, o_hbm,
            x_s, wqkv_s, wo_s, o_s, xn_s, k_s, qt_s, vt_s, ot_s, wt_s,
            wg_s, wu_s, wd_s, pc_s, r_s, y_s, idx_s, fsems, xsems, wsems, osems):
    S, D, H, DH, F, BQ, CK = _S, _D, _H, _DH, _F, _BQ, _CK
    nq, nc, nrc = S // BQ, S // CK, S // _RC

    fcp = [pltpu.make_async_copy(wg_hbm, wg_s, fsems.at[0]),
           pltpu.make_async_copy(wu_hbm, wu_s, fsems.at[1]),
           pltpu.make_async_copy(wd_hbm, wd_s, fsems.at[2])]
    xcp = [pltpu.make_async_copy(x_hbm.at[pl.ds(i * _RC, _RC)], x_s.at[pl.ds(i * _RC, _RC)], xsems.at[i])
           for i in range(nrc)]
    wcp = [pltpu.make_async_copy(wqkv_hbm.at[:, pl.ds(i * D, D)], wqkv_s.at[:, pl.ds(i * D, D)], wsems.at[i])
           for i in range(3)]
    wocp = pltpu.make_async_copy(wo_hbm, wo_s, wsems.at[3])

    def layernorm(i):
        rows = pl.ds(i * _RC, _RC)
        xf = x_s[rows, :].astype(f32)
        mean = jnp.sum(xf, axis=-1, keepdims=True) * (1.0 / D)
        xc0 = xf - mean
        var = jnp.sum(xc0 * xc0, axis=-1, keepdims=True) * (1.0 / D)
        xc = _rb(xf - _rb(mean))
        den = _rb(jnp.sqrt(_rb(_rb(var) + _EPS_BF16)))
        xn_s[rows, :] = (xc * (1.0 / den)).astype(bf16)

    def project(i):
        rows = pl.ds(i * _RC, _RC)
        qv = jax.lax.dot_general(wt_s[...], xn_s[rows, :], (((1,), (1,)), ((), ())),
                                 preferred_element_type=f32)
        qt_s[:, rows] = (qv[0:D] * ((DH ** -0.5) * _LOG2E)).astype(bf16)
        vt_s[:, rows] = qv[D:2 * D].astype(bf16)
        r_s[:, rows] = qv[2 * D:2 * D + 8]

    xcp[0].start()
    for c in wcp:
        c.start()
    xcp[0].wait()
    layernorm(0)
    for c in wcp:
        c.wait()
    for c in xcp[1:]:
        c.start()
    wt_s[0:D, :] = wqkv_s[:, 0:D].T
    wt_s[D:2 * D, :] = wqkv_s[:, 2 * D:3 * D].T
    wt_s[2 * D:2 * D + 16, :] = jnp.broadcast_to(wr_ref[...].reshape(1, D), (16, D))
    project(0)
    for c in xcp[1:]:
        c.wait()
    wocp.start()
    for c in fcp:
        c.start()
    layernorm(1)
    for i in range(1, nrc):
        if i + 1 < nrc:
            layernorm(i + 1)
        project(i)

    for c in fcp:
        c.wait()
    r = _rb(r_s[...])
    rmax = jnp.max(r)
    lane = jax.lax.broadcasted_iota(jnp.int32, (8, S), 1)
    idx = jnp.min(jnp.where(r == rmax, lane, S - 1))
    idx_s[0] = idx
    base = pl.multiple_of((idx // 16) * 16, 16)
    xt = xn_s[pl.ds(base, 16), :]
    row16 = jax.lax.broadcasted_iota(jnp.int32, (16, D), 0)
    xt = jnp.where(row16 == idx - base, xt, jnp.zeros_like(xt))
    groups = [(o, min(512, F - o)) for o in range(0, F, 512)]
    st = {}

    def gate_up(w, name, gi, kk):
        o, n = groups[gi]
        t = _dot(xt[:, kk * 128:(kk + 1) * 128], w[kk * 128:(kk + 1) * 128, o:o + n])
        st[name, gi] = t if kk == 0 else st[name, gi] + t
        if name == "u" and kk == 3:
            g, u = _rb(st["g", gi]), _rb(st["u", gi])
            st["h", gi] = (_rb(g * jax.nn.sigmoid(g)) * u).astype(bf16)

    def down(t):
        gi, o = t // 4, (t % 4) * 128
        p = _dot(st["h", gi][:, o:o + 128], wd_s[t * 128:(t + 1) * 128, :])
        st["y"] = p if t == 0 else st["y"] + p

    fops = []
    for gi in range(len(groups)):
        for w, name in ((wg_s, "g"), (wu_s, "u")):
            for kk in range(4):
                fops.append(functools.partial(gate_up, w, name, gi, kk))
        if gi >= 1:
            fops.extend(functools.partial(down, t) for t in range(4 * (gi - 1), 4 * gi))
    fops.extend(functools.partial(down, t) for t in range(4 * (len(groups) - 1), F // 128))
    kops = [(ci, kk) for ci in range(S // _KC) for kk in range(4)]
    done, kacc = 0, None
    for n, (ci, kk) in enumerate(kops):
        rows = pl.ds(ci * _KC, _KC)
        t = _dot(xn_s[rows, kk * 128:(kk + 1) * 128], wqkv_s[kk * 128:(kk + 1) * 128, D:2 * D])
        kacc = t if kk == 0 else kacc + t
        if kk == 3:
            k_s[rows, :] = kacc.astype(bf16)
        while done < min(((n - 3) * len(fops)) // (len(kops) - 6), len(fops)):
            fops[done]()
            done += 1
    assert done == len(fops)
    y = _rb(st["y"]) * _rb(jax.nn.sigmoid(jnp.full((1, D), rmax, f32)))
    y_s[...] = jnp.broadcast_to(jnp.sum(y, axis=0, keepdims=True), (8, D))

    def qtile(h, joff):
        q16 = qt_s[pl.ds(pl.multiple_of(h * DH, DH), DH), pl.ds(joff, BQ)]
        row = jax.lax.broadcasted_iota(jnp.int32, (128, BQ), 0)
        qf = jnp.concatenate([q16] * 8, axis=0)
        return jnp.where((row // DH) == (h % 8), qf, jnp.zeros_like(qf))

    blocks = [(hl, j) for hl in range(_HPI) for j in range(nq)]
    work = [(b, c) for b in blocks for c in range(nc)]
    nw = len(work)

    def finish(hoff, j, acc, l, bad):
        lt = jnp.sum(l, axis=0, keepdims=True)
        ot_s[pl.ds(hoff, DH), pl.ds(j * BQ, BQ)] = (acc * (1.0 / lt)).astype(bf16)
        ok = jnp.logical_and(lt < _L_MAX, jnp.max(jnp.abs(acc), axis=0, keepdims=True) < np.inf)
        return jnp.maximum(bad, jnp.where(ok, 0.0, 1.0))

    def drain(hprev, acc, l, bad, t):
        hoff = pl.multiple_of(hprev * DH, DH)
        c = nc - _SKEW + t
        acc = acc + _dot(vt_s[pl.ds(hoff, DH), pl.ds(c * CK, CK)], pc_s[t])
        if c == nc - 1:
            bad = finish(hoff, nq - 1, acc, l, bad)
        return acc, bad

    def heads(it, carry):
        bad, acc_p, l_p = carry
        pend = []
        qm, m, l, acc = {}, {}, {}, {}
        hprev = jnp.maximum(it * _HPI - 1, 0)
        for n in range(nw):
            b, c = work[n]
            h = it * _HPI + b[0]
            if b not in qm:
                qm[b] = qtile(h, b[1] * BQ)
            goff = pl.multiple_of((h // 8) * 128, 128)
            s = _dot(k_s[pl.ds(c * CK, CK), pl.ds(goff, 128)], qm[b])
            if c == 0:
                m[b] = jnp.max(jnp.max(s[:_MK].reshape(_MK // 8, 8, BQ), axis=0), axis=0, keepdims=True)
            p = jnp.exp2(s - m[b])
            lc = jnp.sum(p.reshape(CK // 8, 8, BQ), axis=0)
            l[b] = lc if c == 0 else l[b] + lc
            pend.append(p.astype(bf16))
            if n < _SKEW:
                acc_p, bad = drain(hprev, acc_p, l_p, bad, n)
            else:
                b, c = work[n - _SKEW]
                hoff = pl.multiple_of((it * _HPI + b[0]) * DH, DH)
                o = _dot(vt_s[pl.ds(hoff, DH), pl.ds(c * CK, CK)], pend[n - _SKEW])
                acc[b] = o if c == 0 else acc[b] + o
                if c == nc - 1:
                    bad = finish(hoff, b[1], acc[b], l[b], bad)
        for t in range(_SKEW):
            pc_s[t] = pend[nw - _SKEW + t]
        return bad, acc[blocks[-1]], l[blocks[-1]]

    pc_s[...] = jnp.zeros(pc_s.shape, bf16)
    wocp.wait()
    bad, acc_p, l_p = jax.lax.fori_loop(
        0, H // _HPI, heads,
        (jnp.zeros((1, BQ), f32), jnp.zeros((DH, BQ), f32), jnp.ones((8, BQ), f32)))
    for t in range(_SKEW):
        acc_p, bad = drain(H - 1, acc_p, l_p, bad, t)

    @pl.when(jnp.max(bad) > 0.0)
    def _():
        def blk(n, carry):
            h = n // nq
            goff = pl.multiple_of((h // 8) * 128, 128)
            hoff = pl.multiple_of(h * DH, DH)
            joff = pl.multiple_of((n % nq) * BQ, BQ)
            qm = qtile(h, joff)

            def scores(c):
                coff = pl.multiple_of(c * CK, CK)
                return coff, _dot(k_s[pl.ds(coff, CK), pl.ds(goff, 128)], qm)

            def row_max(c, m):
                return jnp.maximum(m, jnp.max(scores(c)[1], axis=0, keepdims=True))
            m = jax.lax.fori_loop(0, nc, row_max, jnp.full((1, BQ), -np.inf, f32))

            def accumulate(c, la):
                coff, s = scores(c)
                p = jnp.exp2(s - m)
                return (la[0] + jnp.sum(p, axis=0, keepdims=True),
                        la[1] + _dot(vt_s[pl.ds(hoff, DH), pl.ds(coff, CK)], p.astype(bf16)))
            l, acc = jax.lax.fori_loop(0, nc, accumulate,
                                       (jnp.zeros((1, BQ), f32), jnp.zeros((DH, BQ), f32)))
            ot_s[pl.ds(hoff, DH), pl.ds(joff, BQ)] = (acc * (1.0 / l)).astype(bf16)
            return carry
        jax.lax.fori_loop(0, H * nq, blk, 0)

    yrow = y_s[0:1, :]
    idx = idx_s[0]
    ocp = [pltpu.make_async_copy(o_s.at[pl.ds(i * _OC, _OC)], o_hbm.at[pl.ds(i * _OC, _OC)], osems.at[i])
           for i in range(S // _OC)]
    for i in range(S // _OC):
        rows = pl.ds(i * _OC, _OC)
        a = jax.lax.dot_general(ot_s[:, rows], wo_s[...], (((0,), (0,)), ((), ())),
                                preferred_element_type=f32)
        row = jax.lax.broadcasted_iota(jnp.int32, (_OC, D), 0)
        upd = jnp.where(row == idx - i * _OC, yrow, 0.0)
        o_s[rows, :] = ((x_s[rows, :].astype(f32) + a) + (xn_s[rows, :].astype(f32) + upd)).astype(bf16)
        ocp[i].start()
    for c in ocp:
        c.wait()


@jax.jit
def pallas_parallel_sum__softmax_full_mha__moe_arch_mod__prompt_kernel(
    A_x: jax.Array,
    A_wqkv: jax.Array,
    A_wo: jax.Array,
    B_x: jax.Array,
    B_w_r: jax.Array,
    B_w_gate: jax.Array,
    B_w_up: jax.Array,
    B_w_down: jax.Array,
):
    S, D, F = _S, _D, _F
    vm = pl.BlockSpec(memory_space=pltpu.VMEM)
    hb = pl.BlockSpec(memory_space=pl.ANY)
    out = pl.pallas_call(
        _kernel,
        out_shape=jax.ShapeDtypeStruct((S, D), bf16),
        in_specs=[hb, hb, hb, vm, hb, hb, hb],
        out_specs=hb,
        scratch_shapes=[
            pltpu.VMEM((S, D), bf16),
            pltpu.VMEM((D, 3 * D), bf16),
            pltpu.VMEM((D, D), bf16),
            pltpu.VMEM((S, D), bf16),
            pltpu.VMEM((S, D), bf16),
            pltpu.VMEM((S, D), bf16),
            pltpu.VMEM((D, S), bf16),
            pltpu.VMEM((D, S), bf16),
            pltpu.VMEM((D, S), bf16),
            pltpu.VMEM((2 * D + 16, D), bf16),
            pltpu.VMEM((D, F), bf16),
            pltpu.VMEM((D, F), bf16),
            pltpu.VMEM((F, D), bf16),
            pltpu.VMEM((_SKEW, _CK, _BQ), bf16),
            pltpu.VMEM((8, S), f32),
            pltpu.VMEM((8, D), f32),
            pltpu.SMEM((1,), jnp.int32),
            pltpu.SemaphoreType.DMA((3,)),
            pltpu.SemaphoreType.DMA((S // _RC,)),
            pltpu.SemaphoreType.DMA((4,)),
            pltpu.SemaphoreType.DMA((S // _OC,)),
        ],
        compiler_params=pltpu.CompilerParams(vmem_limit_bytes=100 * 1024 * 1024),
    )(A_x.reshape(S, D), A_wqkv, A_wo, B_w_r, B_w_gate, B_w_up, B_w_down)
    return out.reshape(1, S, D)
```
